```python
import jax
import jax.numpy as jnp

def _softmax(x, axis=-1):
    return jax.nn.softmax(x, axis=axis)
def _gelu(x):
    return jax.nn.gelu(x, approximate=True)
def _silu(x):
    return jax.nn.silu(x)
def _sigmoid(x):
    return jax.nn.sigmoid(x)
def _layernorm(x, axis=-1, eps=1e-5):
    m = jnp.mean(x, axis=axis, keepdims=True)
    v = jnp.var(x, axis=axis, keepdims=True)
    return (x - m) / jnp.sqrt(v + eps)
def _scatter_add(tgt, idx, src, axis=0):
    return tgt.at[idx].add(src)
def _segment_sum(src, seg, n):
    return jax.ops.segment_sum(src, seg, n)
class _Rng:
    def __init__(self, key):
        self._k = key
    def _next(self):
        self._k, sub = jax.random.split(self._k)
        return sub
    def normal(self, shape):
        return jax.random.normal(self._next(), shape, dtype=jnp.bfloat16)
    def randint(self, lo, hi, shape):
        return jax.random.randint(self._next(), shape, lo, hi, dtype=jnp.int32)
    def uniform(self, shape, lo=0.0, hi=1.0):
        return jax.random.uniform(self._next(), shape, jnp.bfloat16, lo, hi)
    def permutation(self, n):
        return jax.random.permutation(self._next(), n)


kernel_name = 'gated_mix__gqa_block_cached__dense_activation_relu__decode'

def _fwd_setup_inputs():
    _rng = _Rng(jax.random.key(int.from_bytes(__import__("os").urandom(4), "little")))
    _w = (lambda a: (lambda t: t.astype(jnp.bfloat16) if jnp.issubdtype(t.dtype, jnp.floating) else t)(jnp.asarray(a)))
    def _A_setup():
        B, Sq, D = 2, 1, 512
        Hq, Hkv, Sk, Dh = 32, 8, 8192, 128
        assert Hq % Hkv == 0, (Hq, Hkv)
        return {
            "x": _w((lambda *s: _rng.normal(s) * 0.05)(B, Sq, D)),
            "k_cache": _w((lambda *s: _rng.normal(s) * 0.05)(B, Hkv, Sk, Dh)),
            "v_cache": _w((lambda *s: _rng.normal(s) * 0.05)(B, Hkv, Sk, Dh)),
            "wq": _w((lambda *s: _rng.normal(s) * 0.05)(D, Hq * Dh) * (D ** -0.5)),
            "wo": _w((lambda *s: _rng.normal(s) * 0.05)(Hq * Dh, D) * ((Hq * Dh) ** -0.5)),
        }
    _A_in = _A_setup()

    def _B_setup():
        B, S, D, Dff = 2, 1, 512, 1792
        return {
            "x": _w((lambda *s: _rng.normal(s) * 0.05)(B, S, D)),
            "w1": _w((lambda *s: _rng.normal(s) * 0.05)(D, Dff)),
            "w2": _w((lambda *s: _rng.normal(s) * 0.05)(Dff, D)),
        }
    _B_in = _B_setup()

    return {
        "A_x": _A_in["x"],
        "A_k_cache": _A_in["k_cache"],
        "A_v_cache": _A_in["v_cache"],
        "A_wq": _A_in["wq"],
        "A_wo": _A_in["wo"],
        "B_x": _B_in["x"],
        "B_w1": _B_in["w1"],
        "B_w2": _B_in["w2"],
        "gate_w": _w((lambda *s: _rng.normal(s) * 0.05)(512)),
    }

def _fwd_reference(A_x, A_k_cache, A_v_cache, A_wq, A_wo, B_x, B_w1, B_w2, gate_w):
    def _A_ref(x, k_cache, v_cache, wq, wo):
        B, Sq, D = x.shape
        Hq, Dh = 32, 128
        Hkv = k_cache.shape[1]
        rep = Hq // Hkv
        q = (lambda x, *d: x.transpose(*d))((x @ wq).reshape(B, Sq, Hq, Dh), 0, 2, 1, 3)
        k = jnp.repeat(k_cache, rep, axis=1)
        v = jnp.repeat(v_cache, rep, axis=1)
        scores = jnp.einsum("bhqd,bhkd->bhqk", q, k) * (Dh ** -0.5)
        p = _softmax(scores, axis=-1)
        o = jnp.einsum("bhqk,bhkd->bhqd", p, v)
        return (lambda x, *d: x.transpose(*d))(o, 0, 2, 1, 3).reshape(B, Sq, Hq * Dh) @ wo

    def _B_ref(x, w1, w2):
        h = jnp.einsum("bsd,df->bsf", x, w1)
        zero = jnp.zeros_like(h)
        h = jnp.maximum(h, zero)
        return jnp.einsum("bsf,fd->bsd", h, w2)

    x = A_x
    g = _sigmoid((x * gate_w).sum(-1, keepdims=True))
    a = _A_ref(x, A_k_cache, A_v_cache, A_wq, A_wo)
    b = _B_ref(x, B_w1, B_w2)
    return g * a + (1 - g) * b


def setup_inputs():
    _inp = _fwd_setup_inputs()
    _gk = jax.random.fold_in(jax.random.key(int.from_bytes(__import__("os").urandom(4), "little")), 2**31 - 1)
    _shapes = [[2, 1, 512]]
    _dtypes = ['bfloat16']
    _gks = jax.random.split(_gk, len(_shapes))
    _gs = [jax.random.normal(k, s, dtype=jnp.dtype(d)) * 0.05 for k, s, d in zip(_gks, _shapes, _dtypes)]
    _inp["grad_out"] = _gs[0]
    return _inp

def reference(A_x, A_k_cache, A_v_cache, A_wq, A_wo, B_w1, B_w2, gate_w, B_x, grad_out):
    _const = dict(B_x=B_x)
    def _f(*_d):
        return _fwd_reference(**{'A_x': _d[0], 'A_k_cache': _d[1], 'A_v_cache': _d[2], 'A_wq': _d[3], 'A_wo': _d[4], 'B_w1': _d[5], 'B_w2': _d[6], 'gate_w': _d[7], **_const})
    _out, _vjp = jax.vjp(_f, A_x, A_k_cache, A_v_cache, A_wq, A_wo, B_w1, B_w2, gate_w)
    _grads = _vjp(grad_out)
    _out0 = jnp.asarray(_out)
    return (_out0, *[jnp.asarray(_g) for _g in _grads])
```

```python
import jax
import jax.numpy as jnp
from jax import lax
import jax.experimental.pallas as pl
import jax.experimental.pallas.tpu as pltpu

F32 = jnp.float32
BF16 = jnp.bfloat16

NB, D, HQ, HKV, SK, DH, DFF = 2, 512, 32, 8, 8192, 128, 1792
REP = HQ // HKV
GW = REP * DH
SCALE = DH ** -0.5

NN = (((1,), (0,)), ((), ()))
NT = (((1,), (1,)), ((), ()))
TN = (((0,), (0,)), ((), ()))


def _dot(a, b, dims):
    return lax.dot_general(a, b, dims, preferred_element_type=F32)


def _blk(i, n):
    return pl.ds(pl.multiple_of(i * n, n), n)


def _loop(lo, hi, fn):
    if hi > lo:
        lax.fori_loop(lo, hi, lambda j, c: (fn(j), c)[1], 0)


def make(name="fused", ch1=2048, ch2=2048, R=128, pat="m1", wmode="sep", tail=256,
         A=8, Ro=16, Wq=1024, A1=2, order=None, do_dma=True, do_compute=True,
         nosem=False, nobounds=False, wpos=8, first=64):
    SLAB = 4096
    if pat == "m1":
        kv_shape = (4, 8, SLAB, DH)
        head_of = lambda t: t
        slab_idx = lambda s, j: ((0, 2, 1, 3)[s], slice(None), _blk(j, R))

        def place(t, b, c, ch):
            per = SLAB // ch
            return (2 * b + lax.div(t, 4), 2 * lax.rem(t, 4) + lax.div(c, per), _blk(lax.rem(c, per), ch))

        def head_idx(t, b):
            return (2 * b + t // 4, pl.ds(2 * (t % 4), 2))
    else:
        kv_shape = (1, 8, 4 * SLAB, DH)
        head_of = lambda t: 2 * lax.rem(t, 4) + lax.div(t, 4)
        slab_idx = lambda s, j: (0, slice(None), _blk(s * (SLAB // R) + j, R))

        def place(t, b, c, ch):
            return (0, 4 * b + lax.rem(t, 4), _blk(lax.div(t, 4) * (SK // ch) + c, ch))

        def head_idx(t, b):
            return (0, 4 * b + t % 4, _blk(t // 4, SK))
    if order is None:
        order = ["k0", "v0", "k1", "v1", "k2", "v2", "k3", "v3"] if pat == "m1" else \
                ["k0", "k1", "v0", "v1", "v2", "v3", "k2", "k3"]
    NJ = SLAB // R
    sep = wmode == "sep"
    dwq_shape = (A, D // A, HQ * DH) if sep else (D, HQ * DH)
    dwo_shape = (A, HQ * DH // A, D) if sep else (HQ * DH, D)
    dw1_shape = (A1, D // A1, DFF) if sep else (D, DFF)
    dw2_shape = (A1, DFF // A1, D) if sep else (DFF, D)

    def kernel(x_hbm, k_hbm, v_hbm, wq_hbm, wo_hbm, w1_hbm, w2_hbm, gw_hbm, go_hbm,
               out_hbm, dx_hbm, dk_hbm, dv_hbm, dwq_hbm, dwo_hbm, dw1_hbm, dw2_hbm, dgw_hbm,
               kb, vb, wq, wo, w1, w2, dwq, dwo, dw1, dw2,
               xb, gwb, gob, outb, dxb, dgwb, s_ref, dp_ref, ps_ref, q_ref, do_ref, o_ref, dq_ref,
               rsem, wsem):
        cp = pltpu.make_async_copy

        def kv_reads(t):
            return [cp(src.at[head_idx(t, b)], dst.at[head_idx(t, b)], rsem.at[t])
                    for src, dst in ((k_hbm, kb), (v_hbm, vb)) for b in range(NB)]

        def att_reads():
            return [cp(src, dst, rsem.at[HKV]) for src, dst in
                    ((wq_hbm, wq), (x_hbm, xb), (gw_hbm, gwb), (go_hbm, gob), (wo_hbm, wo))]

        def ffn_reads():
            main = pl.ds(0, DFF - tail)
            return [cp(w1_hbm, w1, rsem.at[HKV + 1]), cp(w2_hbm.at[main], w2.at[main], rsem.at[HKV + 1])]

        def last_read():
            rest = pl.ds(DFF - tail, tail)
            return cp(w2_hbm.at[rest], w2.at[rest], rsem.at[HKV + 2])

        def mixed_piece(t):
            cp(dwo.at[_blk(t, 32)], dwo_hbm.at[_blk(t, 32)], wsem).start()
            idx = (_blk(lax.div(t, 2), 8), _blk(lax.rem(t, 2), 2048))
            cp(dwq.at[idx], dwq_hbm.at[idx], wsem).start()

            @pl.when(t < 64)
            def _():
                cp(dw1.at[_blk(t, 8)], dw1_hbm.at[_blk(t, 8)], wsem).start()

            @pl.when(jnp.logical_and(t >= 64, t < 120))
            def _():
                u = jnp.clip(t - 64, 0, 55)
                cp(dw2.at[_blk(u, 32)], dw2_hbm.at[_blk(u, 32)], wsem).start()

        def issue(lo, hi):
            for n, item in enumerate(order):
                src, dst = (kb, dk_hbm) if item[0] == "k" else (vb, dv_hbm)
                s = int(item[1])

                def one(j, src=src, dst=dst, s=s, n=n):
                    cp(src.at[slab_idx(s, j)], dst.at[slab_idx(s, j)], wsem).start()
                    if not sep and n >= 4:
                        per = NJ // 32
                        if per == 1:
                            mixed_piece((n - 4) * 32 + j)
                        else:
                            pl.when(lax.rem(j, per) == 0)(lambda: mixed_piece((n - 4) * 32 + lax.div(j, per)))
                _loop(max(lo - n * NJ, 0), min(hi - n * NJ, NJ), one)

        def weight_writes():
            nc = HQ * DH // Wq

            def fo(j):
                idx = (slice(None), _blk(j, Ro))
                cp(dwo.at[idx], dwo_hbm.at[idx], wsem).start()

            def fq(j):
                idx = (slice(None), _blk(lax.div(j, nc), 8), _blk(lax.rem(j, nc), Wq))
                cp(dwq.at[idx], dwq_hbm.at[idx], wsem).start()

            def f1(j):
                idx = (slice(None), _blk(j, 8))
                cp(dw1.at[idx], dw1_hbm.at[idx], wsem).start()

            def f2(j):
                idx = (slice(None), _blk(j, 32))
                cp(dw2.at[idx], dw2_hbm.at[idx], wsem).start()
            _loop(0, HQ * DH // A // Ro, fo)
            _loop(0, D // A // 8 * nc, fq)
            _loop(0, D // A1 // 8, f1)
            _loop(0, DFF // A1 // 32, f2)

        if do_dma:
            for c in att_reads():
                c.start()
            for t in range(HKV):
                for c in kv_reads(t):
                    c.start()
            for c in ffn_reads():
                c.start()
            if tail:
                last_read().start()
            for c in att_reads():
                c.wait()

        row = lax.broadcasted_iota(jnp.int32, (8, D), 0)
        lo = row < REP

        def rep8(ref):
            v = ref[...].astype(F32)
            return jnp.where(lo, jnp.broadcast_to(v[0:1], (8, D)), jnp.broadcast_to(v[1:2], (8, D)))

        x8 = rep8(xb)
        go8 = rep8(gob)
        gw = gwb[...].astype(F32).reshape(1, D)
        g = jax.nn.sigmoid(jnp.sum(x8 * gw, axis=-1, keepdims=True))
        x8b = x8.astype(BF16)
        da8 = (g * go8).astype(BF16)
        db8 = ((1.0 - g) * go8).astype(BF16)

        col = lax.broadcasted_iota(jnp.int32, (8, GW), 1)
        own = (col // DH) == (row % REP)
        lo1 = lax.broadcasted_iota(jnp.int32, (8, DH), 0) < REP

        def gather_heads(t):
            t = jnp.where(own, t, 0.0)
            return t[:, 0:DH] + t[:, DH:2 * DH] + t[:, 2 * DH:3 * DH] + t[:, 3 * DH:4 * DH]

        def scatter_heads(t):
            return jnp.where(own, jnp.concatenate([t] * REP, axis=1), 0.0)

        def project(h):
            cols = _blk(h, GW)
            q_ref[h] = gather_heads(_dot(x8b, wq[:, cols], NN))
            do_ref[h] = gather_heads(_dot(da8, wo[cols, :], NT))
        if do_compute:
            _loop(0, HKV, project)

        unit = 128 // R

        def step(t):
            last = t == HKV - 1
            if do_dma:
                for c in kv_reads(t):
                    c.wait()

                @pl.when(last)
                def _():
                    for c in ffn_reads():
                        c.wait()
                    issue(0, first)
            if not do_compute:
                return
            h = head_of(t)
            q8, do8 = q_ref[h], do_ref[h]
            q8b, do8b = q8.astype(BF16), do8.astype(BF16)

            def scores(c):
                i0, i1 = place(t, 0, c, ch1), place(t, 1, c, ch1)
                m = lax.broadcasted_iota(jnp.int32, (8, ch1), 0) < REP
                s_ref[:, _blk(c, ch1)] = jnp.where(m, _dot(q8b, kb[i0], NT), _dot(q8b, kb[i1], NT))
                dp_ref[:, _blk(c, ch1)] = jnp.where(m, _dot(do8b, vb[i0], NT), _dot(do8b, vb[i1], NT))
            _loop(0, SK // ch1, scores)

            s = s_ref[...] * SCALE
            e = jnp.exp(s - jnp.max(s, axis=-1, keepdims=True))
            p = e * (1.0 / jnp.sum(e, axis=-1, keepdims=True))
            dp = dp_ref[...]
            ds = p * (dp - jnp.sum(p * dp, axis=-1, keepdims=True)) * SCALE
            ps_ref[...] = jnp.concatenate([p, ds], axis=0).astype(BF16)

            if do_dma:
                pl.when(last)(lambda: issue(first, first + 10 * unit))

            z = jnp.zeros((8, DH), F32)
            wv0 = jnp.concatenate([jnp.where(lo1, do8, 0.0), z], axis=0).astype(BF16)
            wv1 = jnp.concatenate([jnp.where(lo1, 0.0, do8), z], axis=0).astype(BF16)
            wk0 = jnp.concatenate([z, jnp.where(lo1, q8, 0.0)], axis=0).astype(BF16)
            wk1 = jnp.concatenate([z, jnp.where(lo1, 0.0, q8)], axis=0).astype(BF16)

            def grads(c, carry):
                o8, dq8 = carry
                i0, i1 = place(t, 0, c, ch2), place(t, 1, c, ch2)
                ps = ps_ref[:, _blk(c, ch2)]
                o8 = o8 + jnp.where(lo1, _dot(ps, vb[i0], NN)[:8], _dot(ps, vb[i1], NN)[:8])
                dq8 = dq8 + jnp.where(lo1, _dot(ps, kb[i0], NN)[8:], _dot(ps, kb[i1], NN)[8:])
                pst = ps.T
                vb[i0] = _dot(pst, wv0, NN).astype(BF16)
                vb[i1] = _dot(pst, wv1, NN).astype(BF16)
                kb[i0] = _dot(pst, wk0, NN).astype(BF16)
                kb[i1] = _dot(pst, wk1, NN).astype(BF16)
                return o8, dq8
            o_ref[h], dq_ref[h] = lax.fori_loop(0, SK // ch2, grads, (z, z))

        _loop(0, HKV, step)
        n1 = first + 10 * unit if do_compute else first
        n2 = n1 + 20 * unit
        n3 = n2 + 20 * unit
        if do_dma:
            issue(n1, n2)

        if do_compute:
            def unproject(h, carry):
                a8, dxa8 = carry
                cols = _blk(h, GW)
                om = scatter_heads(o_ref[h]).astype(BF16)
                dqm = scatter_heads(dq_ref[h]).astype(BF16)
                a8 = a8 + _dot(om, wo[cols, :], NN)
                dxa8 = dxa8 + _dot(dqm, wq[:, cols], NT)
                dwo_h = _dot(om, da8, TN).astype(BF16)
                dwq_h = _dot(x8b, dqm, TN).astype(BF16)
                if sep:
                    per = HQ * DH // A // GW
                    dwo[lax.div(h, per), _blk(lax.rem(h, per), GW), :] = dwo_h
                    dwq[:, :, cols] = dwq_h.reshape(A, D // A, GW)
                else:
                    dwo[cols, :] = dwo_h
                    dwq[:, cols] = dwq_h
                return a8, dxa8
            zero8 = jnp.zeros((8, D), F32)
            a8, dxa8 = lax.fori_loop(0, HKV, unproject, (zero8, zero8))

        if do_dma:
            issue(n2, n3)
            if tail:
                last_read().wait()

        if do_compute:
            first_row = (row % REP) == 0
            hid = _dot(x8b, w1[...], NN)
            r8 = jnp.maximum(hid, 0.0).astype(BF16)
            b8 = _dot(r8, w2[...], NN)
            dr = _dot(db8, w2[...], NT)
            dh = (dr * jnp.where(hid > 0.0, 1.0, jnp.where(hid == 0.0, 0.5, 0.0))).astype(BF16)
            dxf8 = _dot(dh, w1[...], NT)
            dw1[...] = _dot(jnp.where(first_row, x8, 0.0).astype(BF16), dh, TN).astype(BF16).reshape(dw1_shape)
            dw2[...] = _dot(r8, jnp.where(first_row, db8.astype(F32), 0.0).astype(BF16), TN).astype(BF16).reshape(dw2_shape)

            def per_token(t8):
                t0 = jnp.sum(jnp.where(lo, t8, 0.0), axis=0, keepdims=True)
                t1 = jnp.sum(jnp.where(lo, 0.0, t8), axis=0, keepdims=True)
                return jnp.concatenate([t0, t1], axis=0)

            a = per_token(a8)
            dxa = per_token(dxa8)
            b = per_token(jnp.where(first_row, b8, 0.0))
            dxf = per_token(jnp.where(first_row, dxf8, 0.0))
            x2 = xb[...].astype(F32)
            go2 = gob[...].astype(F32)
            g2 = jax.nn.sigmoid(jnp.sum(x2 * gw, axis=-1, keepdims=True))
            outb[...] = (g2 * a + (1.0 - g2) * b).astype(BF16)
            dz = jnp.sum(go2 * (a - b), axis=-1, keepdims=True) * g2 * (1.0 - g2)
            dxb[...] = (dxa + dxf + dz * gw).astype(BF16)
            dgwb[...] = jnp.sum(dz * x2, axis=0).astype(BF16)

        if do_dma:
            small = (cp(outb, out_hbm, wsem), cp(dxb, dx_hbm, wsem), cp(dgwb, dgw_hbm, wsem))
            for c in small:
                c.start()
            cut = max(n3, wpos * NJ)
            issue(n3, cut)
            if sep:
                weight_writes()
            issue(cut, 8 * NJ)
            for c in small:
                c.wait()
            for src, dst in ((dwq, dwq_hbm), (dwo, dwo_hbm), (dw1, dw1_hbm), (dw2, dw2_hbm), (kb, dk_hbm), (vb, dv_hbm)):
                cp(src, dst, wsem).wait()

    @jax.jit
    def f(A_x, A_k_cache, A_v_cache, A_wq, A_wo, B_x, B_w1, B_w2, gate_w, grad_out):
        del B_x
        args = (A_x.reshape(NB, D), A_k_cache.reshape(kv_shape), A_v_cache.reshape(kv_shape),
                A_wq, A_wo, B_w1, B_w2, gate_w, grad_out.reshape(NB, D))
        shapes = [(NB, D), (NB, D), kv_shape, kv_shape, dwq_shape, dwo_shape, dw1_shape, dw2_shape, gate_w.shape]
        hbm = pl.BlockSpec(memory_space=pltpu.HBM)
        vm = lambda shape, dt=BF16: pltpu.VMEM(shape, dt)
        res = pl.pallas_call(
            kernel,
            out_shape=[jax.ShapeDtypeStruct(s, BF16) for s in shapes],
            in_specs=[hbm] * len(args),
            out_specs=[hbm] * len(shapes),
            scratch_shapes=[
                vm(kv_shape), vm(kv_shape),
                vm(A_wq.shape), vm(A_wo.shape), vm(B_w1.shape), vm(B_w2.shape),
                vm(dwq_shape), vm(dwo_shape), vm(dw1_shape), vm(dw2_shape),
                vm((NB, D)), vm((D,)), vm((NB, D)), vm((NB, D)), vm((NB, D)), vm((D,)),
                vm((8, SK), F32), vm((8, SK), F32), vm((16, SK)),
                vm((HKV, 8, DH), F32), vm((HKV, 8, DH), F32), vm((HKV, 8, DH), F32), vm((HKV, 8, DH), F32),
                pltpu.SemaphoreType.DMA((HKV + 3,)), pltpu.SemaphoreType.DMA(()),
            ],
            compiler_params=pltpu.CompilerParams(
                vmem_limit_bytes=110 * 2**20,
                disable_semaphore_checks=nosem, disable_bounds_checks=nobounds),
            name=name,
        )(*args)
        out, dx, dk, dv, dwq, dwo, dw1, dw2, dgw = res
        return (out.reshape(A_x.shape), dx.reshape(A_x.shape), dk.reshape(A_k_cache.shape),
                dv.reshape(A_v_cache.shape), dwq.reshape(A_wq.shape), dwo.reshape(A_wo.shape),
                dw1.reshape(B_w1.shape), dw2.reshape(B_w2.shape), dgw)
    return f


_kernel = make(name="gated_mix_gqa_relu_decode", R=64)


@jax.jit
def pallas_gated_mix__gqa_block_cached__dense_activation_relu__decode_kernel(
        A_x, A_k_cache, A_v_cache, A_wq, A_wo, B_x, B_w1, B_w2, gate_w, grad_out):
    return _kernel(A_x, A_k_cache, A_v_cache, A_wq, A_wo, B_x, B_w1, B_w2, gate_w, grad_out)
```

```python
import jax
import jax.numpy as jnp
from jax import lax
import jax.experimental.pallas as pl
import jax.experimental.pallas.tpu as pltpu

F32 = jnp.float32
BF16 = jnp.bfloat16

NB, D, HQ, HKV, SK, DH, DFF = 2, 512, 32, 8, 8192, 128, 1792
REP = HQ // HKV
GW = REP * DH
SCALE = DH ** -0.5

STREAM = SK // 2
KV_VIEW = (2 * NB, HKV, STREAM, DH)
CHUNK = 2048
W_ROWS = 64
DWQ_VIEW = (4, D // 4, HQ * DH)
DWO_VIEW = (4, HQ * DH // 4, D)
TAIL = 448
RING = 3

NN = (((1,), (0,)), ((), ()))
NT = (((1,), (1,)), ((), ()))
TN = (((0,), (0,)), ((), ()))


def _dot(a, b, dims):
    return lax.dot_general(a, b, dims, preferred_element_type=F32)


def _blk(i, n):
    return pl.ds(pl.multiple_of(i * n, n), n)


def _loop(lo, hi, body):
    def step(i, carry):
        body(i)
        return carry
    lax.fori_loop(lo, hi, step, 0)


def _start(copies):
    for c in copies:
        c.start()


def _wait(copies):
    for c in copies:
        c.wait()


def _kernel(x_hbm, k_hbm, v_hbm, wq_hbm, wo_hbm, w1_hbm, w2_hbm, gw_hbm, go_hbm,
            out_hbm, dx_hbm, dk_hbm, dv_hbm, dwq_hbm, dwo_hbm, dw1_hbm, dw2_hbm, dgw_hbm,
            k_ref, v_ref, wq_ref, wo_ref, w1_ref, w2_ref, dwq_ref, dwo_ref, dw1_ref, dw2_ref,
            x_ref, gw_ref, go_ref, out_ref, dx_ref, dgw_ref,
            s_ref, dp_ref, ps_ref, q_ref, do_ref, o_ref, dq_ref, sems):
    copy = pltpu.make_async_copy

    def attn_reads():
        return [copy(src, dst, sems.at[0]) for src, dst in (
            (wq_hbm, wq_ref), (x_hbm, x_ref), (gw_hbm, gw_ref), (go_hbm, go_ref), (wo_hbm, wo_ref))]

    def kv_reads(h):
        sem = sems.at[(h + 1) % RING]
        heads = [(2 * b + h // 4, pl.ds(2 * (h % 4), 2)) for b in range(NB)]
        return [copy(src.at[i], dst.at[i], sem)
                for src, dst in ((k_hbm, k_ref), (v_hbm, v_ref)) for i in heads]

    def ffn_reads():
        sem, rows = sems.at[(HKV + 1) % RING], pl.ds(0, DFF - TAIL)
        return [copy(w1_hbm, w1_ref, sem), copy(w2_hbm.at[rows], w2_ref.at[rows], sem)]

    def tail_read():
        rows = pl.ds(DFF - TAIL, TAIL)
        return [copy(w2_hbm.at[rows], w2_ref.at[rows], sems.at[(HKV + 2) % RING])]

    def write(src, dst, idx):
        return copy(src.at[idx], dst.at[idx], sems.at[HKV % RING])

    def slab_writes(n, act):
        src, dst = ((k_ref, dk_hbm), (v_ref, dv_hbm))[n % 2]
        slab = 2 * (n // 2 % 2) + n // 4
        _loop(0, STREAM // W_ROWS,
              lambda j: act([write(src, dst, (slab, slice(None), _blk(j, W_ROWS)))]))

    def weight_writes(act):
        def pieces(j):
            return [write(dwq_ref, dwq_hbm, (slice(None), _blk(lax.div(j, 4), 8), _blk(lax.rem(j, 4), 1024))),
                    write(dw1_ref, dw1_hbm, (_blk(j, 8),)),
                    write(dwo_ref, dwo_hbm, (slice(None), _blk(j, 16)))]
        _loop(0, DFF // 32, lambda j: act(pieces(j) + [write(dw2_ref, dw2_hbm, (_blk(j, 32),))]))
        _loop(DFF // 32, D // 8, lambda j: act(pieces(j)))

    def small_writes():
        return [copy(src, dst, sems.at[HKV % RING]) for src, dst in (
            (out_ref, out_hbm), (dx_ref, dx_hbm), (dgw_ref, dgw_hbm))]

    _start(attn_reads())
    for h in range(RING - 1):
        _start(kv_reads(h))
    _wait(attn_reads())
    _start(kv_reads(RING - 1))

    x = x_ref[...].astype(F32)
    go = go_ref[...].astype(F32)
    gw = gw_ref[...].astype(F32).reshape(1, D)
    g = jax.nn.sigmoid(jnp.sum(x * gw, axis=-1, keepdims=True))

    row = lax.broadcasted_iota(jnp.int32, (8, D), 0)
    tok0 = row < REP
    first = row % REP == 0

    def spread(t):
        return jnp.where(tok0, jnp.broadcast_to(t[0:1], (8, D)), jnp.broadcast_to(t[1:2], (8, D)))

    def per_token(t):
        return jnp.concatenate([jnp.sum(jnp.where(tok0, t, 0.0), axis=0, keepdims=True),
                                jnp.sum(jnp.where(tok0, 0.0, t), axis=0, keepdims=True)], axis=0)

    x8 = spread(x)
    db8 = spread((1.0 - g) * go)
    x8b = x8.astype(BF16)
    da8b = spread(g * go).astype(BF16)

    own = lax.broadcasted_iota(jnp.int32, (8, GW), 1) // DH == row % REP

    def gather_heads(t):
        t = jnp.where(own, t, 0.0)
        return sum(t[:, i * DH:(i + 1) * DH] for i in range(1, REP)) + t[:, :DH]

    def scatter_heads(t):
        return jnp.where(own, jnp.concatenate([t] * REP, axis=1), 0.0)

    def project(h):
        cols = _blk(h, GW)
        q_ref[h] = gather_heads(_dot(x8b, wq_ref[:, cols], NN))
        do_ref[h] = gather_heads(_dot(da8b, wo_ref[cols, :], NT))
    _loop(0, HKV, project)

    def attend(h):
        last = h == HKV - 1
        _wait(kv_reads(h))
        pl.when(h + RING < HKV)(lambda: _start(kv_reads(jnp.minimum(h + RING, HKV - 1))))
        pl.when(h + RING == HKV)(lambda: _start(ffn_reads()))
        pl.when(h + RING == HKV + 1)(lambda: _start(tail_read()))

        @pl.when(last)
        def _():
            _wait(ffn_reads())
            slab_writes(0, _start)

        def chunk(c):
            per = STREAM // CHUNK
            stream = 2 * lax.rem(h, 4) + lax.div(c, per)
            return [(2 * b + lax.div(h, 4), stream, _blk(lax.rem(c, per), CHUNK)) for b in range(NB)]

        q, do = q_ref[h], do_ref[h]
        qb, dob = q.astype(BF16), do.astype(BF16)

        def scores(c):
            i0, i1 = chunk(c)
            m = lax.broadcasted_iota(jnp.int32, (8, CHUNK), 0) < REP
            s_ref[:, _blk(c, CHUNK)] = jnp.where(m, _dot(qb, k_ref[i0], NT), _dot(qb, k_ref[i1], NT))
            dp_ref[:, _blk(c, CHUNK)] = jnp.where(m, _dot(dob, v_ref[i0], NT), _dot(dob, v_ref[i1], NT))
        _loop(0, SK // CHUNK, scores)

        s = s_ref[...] * SCALE
        e = jnp.exp(s - jnp.max(s, axis=-1, keepdims=True))
        p = e * (1.0 / jnp.sum(e, axis=-1, keepdims=True))
        dp = dp_ref[...]
        ds = p * (dp - jnp.sum(p * dp, axis=-1, keepdims=True)) * SCALE
        ps_ref[...] = jnp.concatenate([p, ds], axis=0).astype(BF16)

        pl.when(last)(lambda: slab_writes(1, _start))

        m = lax.broadcasted_iota(jnp.int32, (8, DH), 0) < REP
        zero = jnp.zeros((8, DH), F32)
        to_dv0 = jnp.concatenate([jnp.where(m, do, 0.0), zero], axis=0).astype(BF16)
        to_dv1 = jnp.concatenate([jnp.where(m, 0.0, do), zero], axis=0).astype(BF16)
        to_dk0 = jnp.concatenate([zero, jnp.where(m, q, 0.0)], axis=0).astype(BF16)
        to_dk1 = jnp.concatenate([zero, jnp.where(m, 0.0, q)], axis=0).astype(BF16)

        def grads(c, carry):
            o, dq = carry
            i0, i1 = chunk(c)
            ps = ps_ref[:, _blk(c, CHUNK)]
            o = o + jnp.where(m, _dot(ps, v_ref[i0], NN)[:8], _dot(ps, v_ref[i1], NN)[:8])
            dq = dq + jnp.where(m, _dot(ps, k_ref[i0], NN)[8:], _dot(ps, k_ref[i1], NN)[8:])
            pst = ps.T
            v_ref[i0] = _dot(pst, to_dv0, NN).astype(BF16)
            v_ref[i1] = _dot(pst, to_dv1, NN).astype(BF16)
            k_ref[i0] = _dot(pst, to_dk0, NN).astype(BF16)
            k_ref[i1] = _dot(pst, to_dk1, NN).astype(BF16)
            return o, dq
        o_ref[h], dq_ref[h] = lax.fori_loop(0, SK // CHUNK, grads, (zero, zero))
    _loop(0, HKV, attend)
    slab_writes(2, _start)

    def unproject(h, carry):
        a8, dx8 = carry
        cols = _blk(h, GW)
        o = scatter_heads(o_ref[h]).astype(BF16)
        dq = scatter_heads(dq_ref[h]).astype(BF16)
        per = DWO_VIEW[1] // GW
        dwo_ref[lax.div(h, per), _blk(lax.rem(h, per), GW), :] = _dot(o, da8b, TN).astype(BF16)
        dwq_ref[:, :, cols] = _dot(x8b, dq, TN).astype(BF16).reshape(*DWQ_VIEW[:2], GW)
        return a8 + _dot(o, wo_ref[cols, :], NN), dx8 + _dot(dq, wq_ref[:, cols], NT)
    zero8 = jnp.zeros((8, D), F32)
    a8, dx8 = lax.fori_loop(0, HKV, unproject, (zero8, zero8))
    slab_writes(3, _start)

    _wait(tail_read())
    hid = _dot(x8b, w1_ref[...], NN)
    act = jnp.maximum(hid, 0.0).astype(BF16)
    b8 = _dot(act, w2_ref[...], NN)
    slope = jnp.where(hid > 0.0, 1.0, jnp.where(hid == 0.0, 0.5, 0.0))
    dhid = (_dot(db8.astype(BF16), w2_ref[...], NT) * slope).astype(BF16)
    dx8 = dx8 + jnp.where(first, _dot(dhid, w1_ref[...], NT), 0.0)
    dw1_ref[...] = _dot(jnp.where(first, x8, 0.0).astype(BF16), dhid, TN).astype(BF16)
    dw2_ref[...] = _dot(act, jnp.where(first, db8, 0.0).astype(BF16), TN).astype(BF16)

    a = per_token(a8)
    b = per_token(jnp.where(first, b8, 0.0))
    dz = jnp.sum(go * (a - b), axis=-1, keepdims=True) * g * (1.0 - g)
    out_ref[...] = (g * a + (1.0 - g) * b).astype(BF16)
    dx_ref[...] = (per_token(dx8) + dz * gw).astype(BF16)
    dgw_ref[...] = jnp.sum(dz * x, axis=0).astype(BF16)

    _start(small_writes())
    weight_writes(_start)
    for n in range(4, 8):
        slab_writes(n, _start)

    for n in range(8):
        slab_writes(n, _wait)
    weight_writes(_wait)
    _wait(small_writes())


@jax.jit
def pallas_gated_mix__gqa_block_cached__dense_activation_relu__decode_kernel(
    A_x: jax.Array,
    A_k_cache: jax.Array,
    A_v_cache: jax.Array,
    A_wq: jax.Array,
    A_wo: jax.Array,
    B_x: jax.Array,
    B_w1: jax.Array,
    B_w2: jax.Array,
    gate_w: jax.Array,
    grad_out: jax.Array,
):
    del B_x
    args = (A_x.reshape(NB, D), A_k_cache.reshape(KV_VIEW), A_v_cache.reshape(KV_VIEW),
            A_wq, A_wo, B_w1, B_w2, gate_w, grad_out.reshape(NB, D))
    grads = (KV_VIEW, KV_VIEW, DWQ_VIEW, DWO_VIEW, B_w1.shape, B_w2.shape)
    out_shapes = ((NB, D), (NB, D), *grads, gate_w.shape)
    hbm = pl.BlockSpec(memory_space=pltpu.HBM)

    out, dx, dk, dv, dwq, dwo, dw1, dw2, dgw = pl.pallas_call(
        _kernel,
        out_shape=[jax.ShapeDtypeStruct(s, BF16) for s in out_shapes],
        in_specs=[hbm] * len(args),
        out_specs=[hbm] * len(out_shapes),
        scratch_shapes=[
            *(pltpu.VMEM(s, BF16) for s in (
                KV_VIEW, KV_VIEW, A_wq.shape, A_wo.shape, B_w1.shape, B_w2.shape, *grads[2:],
                (NB, D), (D,), (NB, D), (NB, D), (NB, D), (D,))),
            pltpu.VMEM((8, SK), F32), pltpu.VMEM((8, SK), F32), pltpu.VMEM((16, SK), BF16),
            *(pltpu.VMEM((HKV, 8, DH), F32) for _ in range(4)),
            pltpu.SemaphoreType.DMA((RING,)),
        ],
        compiler_params=pltpu.CompilerParams(vmem_limit_bytes=110 * 2**20),
        name="gated_mix_gqa_relu_decode",
    )(*args)
    return (out.reshape(A_x.shape), dx.reshape(A_x.shape),
            dk.reshape(A_k_cache.shape), dv.reshape(A_v_cache.shape),
            dwq.reshape(A_wq.shape), dwo.reshape(A_wo.shape), dw1, dw2, dgw)
```

```python
import jax
import jax.numpy as jnp
from jax import lax
import jax.experimental.pallas as pl
import jax.experimental.pallas.tpu as pltpu

F32 = jnp.float32
BF16 = jnp.bfloat16

NB, D, HQ, HKV, SK, DH, DFF = 2, 512, 32, 8, 8192, 128, 1792
REP = HQ // HKV
GW = REP * DH
SCALE = DH ** -0.5

STREAM = SK // 2
KV_VIEW = (2 * NB, HKV, STREAM, DH)
CHUNK = 2048
W_ROWS = 112
DWQ_VIEW = (4, D // 4, HQ * DH)
DWO_VIEW = (4, HQ * DH // 4, D)
DW1_VIEW = (4, D // 4, DFF)
DW2_VIEW = (4, DFF // 4, D)
TAIL = 448
RING = 3

NN = (((1,), (0,)), ((), ()))
NT = (((1,), (1,)), ((), ()))
TN = (((0,), (0,)), ((), ()))
ALL = slice(None)


def _dot(a, b, dims):
    return lax.dot_general(a, b, dims, preferred_element_type=F32)


def _blk(i, n):
    return pl.ds(pl.multiple_of(i * n, n), n)


def _loop(lo, hi, body):
    def step(i, carry):
        body(i)
        return carry
    lax.fori_loop(lo, hi, step, 0)


def _start(copies):
    for c in copies:
        c.start()


def _wait(copies):
    for c in copies:
        c.wait()


def _kernel(x_hbm, k_hbm, v_hbm, wq_hbm, wo_hbm, w1_hbm, w2_hbm, gw_hbm, go_hbm,
            out_hbm, dx_hbm, dk_hbm, dv_hbm, dwq_hbm, dwo_hbm, dw1_hbm, dw2_hbm, dgw_hbm,
            k_ref, v_ref, wq_ref, wo_ref, w1_ref, w2_ref, dwq_ref, dwo_ref, dw1_ref, dw2_ref,
            x_ref, gw_ref, go_ref, out_ref, dx_ref, dgw_ref,
            s_ref, dp_ref, ps_ref, q_ref, do_ref, o_ref, dq_ref, sems):
    copy = pltpu.make_async_copy

    def attn_reads():
        return [copy(src, dst, sems.at[0]) for src, dst in (
            (wq_hbm, wq_ref), (x_hbm, x_ref), (gw_hbm, gw_ref), (go_hbm, go_ref), (wo_hbm, wo_ref))]

    def kv_reads(h):
        sem = sems.at[(h + 1) % RING]
        heads = [(2 * b + h // 4, pl.ds(2 * (h % 4), 2)) for b in range(NB)]
        return [copy(src.at[i], dst.at[i], sem)
                for src, dst in ((k_hbm, k_ref), (v_hbm, v_ref)) for i in heads]

    def ffn_reads():
        sem, rows = sems.at[(HKV + 1) % RING], pl.ds(0, DFF - TAIL)
        return [copy(w1_hbm, w1_ref, sem), copy(w2_hbm.at[rows], w2_ref.at[rows], sem)]

    def tail_read():
        rows = pl.ds(DFF - TAIL, TAIL)
        return [copy(w2_hbm.at[rows], w2_ref.at[rows], sems.at[(HKV + 2) % RING])]

    def write(src, dst, idx):
        return copy(src.at[idx], dst.at[idx], sems.at[HKV % RING])

    def slab_writes(n, act):
        src, dst = ((k_ref, dk_hbm), (v_ref, dv_hbm))[n % 2]
        slab = 2 * (n // 2 % 2) + n // 4
        full, rest = divmod(STREAM, W_ROWS)
        _loop(0, full, lambda j: act([write(src, dst, (slab, ALL, _blk(j, W_ROWS)))]))
        act([write(src, dst, (slab, ALL, pl.ds(full * W_ROWS, rest)))])

    def weight_writes(act):
        def dwq(j):
            return write(dwq_ref, dwq_hbm, (ALL, _blk(lax.div(j, 4), 8), _blk(lax.rem(j, 4), HQ * DH // 4)))

        def dwo(j):
            return write(dwo_ref, dwo_hbm, (ALL, _blk(j, 16)))

        def dw1(j):
            return write(dw1_ref, dw1_hbm, (ALL, _blk(j, 8)))

        def dw2(j):
            return write(dw2_ref, dw2_hbm, (ALL, _blk(j, 32)))

        _loop(0, DWO_VIEW[1] // 16, lambda j: act([dwq(j), dwo(j)]))
        _loop(0, DW2_VIEW[1] // 32, lambda j: act([dw1(j), dw2(j)]))
        _loop(DW2_VIEW[1] // 32, DW1_VIEW[1] // 8, lambda j: act([dw1(j)]))

    def small_writes():
        return [copy(src, dst, sems.at[HKV % RING]) for src, dst in (
            (out_ref, out_hbm), (dx_ref, dx_hbm), (dgw_ref, dgw_hbm))]

    _start(attn_reads())
    for h in range(RING - 1):
        _start(kv_reads(h))
    _wait(attn_reads())
    _start(kv_reads(RING - 1))

    x = x_ref[...].astype(F32)
    go = go_ref[...].astype(F32)
    gw = gw_ref[...].astype(F32).reshape(1, D)
    g = jax.nn.sigmoid(jnp.sum(x * gw, axis=-1, keepdims=True))

    row = lax.broadcasted_iota(jnp.int32, (8, D), 0)
    tok0 = row < REP
    first = row % REP == 0

    def spread(t):
        return jnp.where(tok0, jnp.broadcast_to(t[0:1], (8, D)), jnp.broadcast_to(t[1:2], (8, D)))

    def per_token(t):
        return jnp.concatenate([jnp.sum(jnp.where(tok0, t, 0.0), axis=0, keepdims=True),
                                jnp.sum(jnp.where(tok0, 0.0, t), axis=0, keepdims=True)], axis=0)

    x8 = spread(x)
    db8 = spread((1.0 - g) * go)
    x8b = x8.astype(BF16)
    da8b = spread(g * go).astype(BF16)

    own = lax.broadcasted_iota(jnp.int32, (8, GW), 1) // DH == row % REP

    def gather_heads(t):
        t = jnp.where(own, t, 0.0)
        return sum(t[:, i * DH:(i + 1) * DH] for i in range(1, REP)) + t[:, :DH]

    def scatter_heads(t):
        return jnp.where(own, jnp.concatenate([t] * REP, axis=1), 0.0)

    def project(h):
        cols = _blk(h, GW)
        q_ref[h] = gather_heads(_dot(x8b, wq_ref[:, cols], NN))
        do_ref[h] = gather_heads(_dot(da8b, wo_ref[cols, :], NT))
    _loop(0, HKV, project)

    def attend(h):
        last = h == HKV - 1
        _wait(kv_reads(h))
        pl.when(h + RING < HKV)(lambda: _start(kv_reads(jnp.minimum(h + RING, HKV - 1))))
        pl.when(h + RING == HKV)(lambda: _start(ffn_reads()))
        pl.when(h + RING == HKV + 1)(lambda: _start(tail_read()))

        @pl.when(last)
        def _():
            _wait(ffn_reads())
            slab_writes(0, _start)

        def chunk(c):
            per = STREAM // CHUNK
            stream = 2 * lax.rem(h, 4) + lax.div(c, per)
            return [(2 * b + lax.div(h, 4), stream, _blk(lax.rem(c, per), CHUNK)) for b in range(NB)]

        q, do = q_ref[h], do_ref[h]
        qb, dob = q.astype(BF16), do.astype(BF16)

        def scores(c):
            i0, i1 = chunk(c)
            m = lax.broadcasted_iota(jnp.int32, (8, CHUNK), 0) < REP
            s_ref[:, _blk(c, CHUNK)] = jnp.where(m, _dot(qb, k_ref[i0], NT), _dot(qb, k_ref[i1], NT))
            dp_ref[:, _blk(c, CHUNK)] = jnp.where(m, _dot(dob, v_ref[i0], NT), _dot(dob, v_ref[i1], NT))
        _loop(0, SK // CHUNK, scores)

        s = s_ref[...] * SCALE
        e = jnp.exp(s - jnp.max(s, axis=-1, keepdims=True))
        p = e * (1.0 / jnp.sum(e, axis=-1, keepdims=True))
        dp = dp_ref[...]
        ds = p * (dp - jnp.sum(p * dp, axis=-1, keepdims=True)) * SCALE
        ps_ref[...] = jnp.concatenate([p, ds], axis=0).astype(BF16)

        pl.when(last)(lambda: slab_writes(1, _start))

        m = lax.broadcasted_iota(jnp.int32, (8, DH), 0) < REP
        zero = jnp.zeros((8, DH), F32)
        to_dv0 = jnp.concatenate([jnp.where(m, do, 0.0), zero], axis=0).astype(BF16)
        to_dv1 = jnp.concatenate([jnp.where(m, 0.0, do), zero], axis=0).astype(BF16)
        to_dk0 = jnp.concatenate([zero, jnp.where(m, q, 0.0)], axis=0).astype(BF16)
        to_dk1 = jnp.concatenate([zero, jnp.where(m, 0.0, q)], axis=0).astype(BF16)

        def grads(c, carry):
            o, dq = carry
            i0, i1 = chunk(c)
            ps = ps_ref[:, _blk(c, CHUNK)]
            o = o + jnp.where(m, _dot(ps, v_ref[i0], NN)[:8], _dot(ps, v_ref[i1], NN)[:8])
            dq = dq + jnp.where(m, _dot(ps, k_ref[i0], NN)[8:], _dot(ps, k_ref[i1], NN)[8:])
            pst = ps.T
            v_ref[i0] = _dot(pst, to_dv0, NN).astype(BF16)
            v_ref[i1] = _dot(pst, to_dv1, NN).astype(BF16)
            k_ref[i0] = _dot(pst, to_dk0, NN).astype(BF16)
            k_ref[i1] = _dot(pst, to_dk1, NN).astype(BF16)
            return o, dq
        o_ref[h], dq_ref[h] = lax.fori_loop(0, SK // CHUNK, grads, (zero, zero))
    _loop(0, HKV, attend)
    slab_writes(2, _start)

    def unproject(h, carry):
        a8, dx8 = carry
        cols = _blk(h, GW)
        o = scatter_heads(o_ref[h]).astype(BF16)
        dq = scatter_heads(dq_ref[h]).astype(BF16)
        per = DWO_VIEW[1] // GW
        dwo_ref[lax.div(h, per), _blk(lax.rem(h, per), GW), :] = _dot(o, da8b, TN).astype(BF16)
        dwq_ref[:, :, cols] = _dot(x8b, dq, TN).astype(BF16).reshape(*DWQ_VIEW[:2], GW)
        return a8 + _dot(o, wo_ref[cols, :], NN), dx8 + _dot(dq, wq_ref[:, cols], NT)
    zero8 = jnp.zeros((8, D), F32)
    a8, dx8 = lax.fori_loop(0, HKV, unproject, (zero8, zero8))
    slab_writes(3, _start)

    _wait(tail_read())
    hid = _dot(x8b, w1_ref[...], NN)
    act = jnp.maximum(hid, 0.0).astype(BF16)
    b8 = _dot(act, w2_ref[...], NN)
    slope = jnp.where(hid > 0.0, 1.0, jnp.where(hid == 0.0, 0.5, 0.0))
    dhid = (_dot(db8.astype(BF16), w2_ref[...], NT) * slope).astype(BF16)
    dx8 = dx8 + jnp.where(first, _dot(dhid, w1_ref[...], NT), 0.0)
    dw1_ref[...] = _dot(jnp.where(first, x8, 0.0).astype(BF16), dhid, TN).astype(BF16).reshape(DW1_VIEW)
    dw2_ref[...] = _dot(act, jnp.where(first, db8, 0.0).astype(BF16), TN).astype(BF16).reshape(DW2_VIEW)

    a = per_token(a8)
    b = per_token(jnp.where(first, b8, 0.0))
    dz = jnp.sum(go * (a - b), axis=-1, keepdims=True) * g * (1.0 - g)
    out_ref[...] = (g * a + (1.0 - g) * b).astype(BF16)
    dx_ref[...] = (per_token(dx8) + dz * gw).astype(BF16)
    dgw_ref[...] = jnp.sum(dz * x, axis=0).astype(BF16)

    _start(small_writes())
    weight_writes(_start)
    for n in range(4, 8):
        slab_writes(n, _start)

    for n in range(8):
        slab_writes(n, _wait)
    weight_writes(_wait)
    _wait(small_writes())


@jax.jit
def pallas_gated_mix__gqa_block_cached__dense_activation_relu__decode_kernel(
    A_x: jax.Array,
    A_k_cache: jax.Array,
    A_v_cache: jax.Array,
    A_wq: jax.Array,
    A_wo: jax.Array,
    B_x: jax.Array,
    B_w1: jax.Array,
    B_w2: jax.Array,
    gate_w: jax.Array,
    grad_out: jax.Array,
):
    del B_x
    args = (A_x.reshape(NB, D), A_k_cache.reshape(KV_VIEW), A_v_cache.reshape(KV_VIEW),
            A_wq, A_wo, B_w1, B_w2, gate_w, grad_out.reshape(NB, D))
    grads = (KV_VIEW, KV_VIEW, DWQ_VIEW, DWO_VIEW, DW1_VIEW, DW2_VIEW)
    out_shapes = ((NB, D), (NB, D), *grads, gate_w.shape)
    hbm = pl.BlockSpec(memory_space=pltpu.HBM)

    out, dx, dk, dv, dwq, dwo, dw1, dw2, dgw = pl.pallas_call(
        _kernel,
        out_shape=[jax.ShapeDtypeStruct(s, BF16) for s in out_shapes],
        in_specs=[hbm] * len(args),
        out_specs=[hbm] * len(out_shapes),
        scratch_shapes=[
            *(pltpu.VMEM(s, BF16) for s in (
                KV_VIEW, KV_VIEW, A_wq.shape, A_wo.shape, B_w1.shape, B_w2.shape, *grads[2:],
                (NB, D), (D,), (NB, D), (NB, D), (NB, D), (D,))),
            pltpu.VMEM((8, SK), F32), pltpu.VMEM((8, SK), F32), pltpu.VMEM((16, SK), BF16),
            *(pltpu.VMEM((HKV, 8, DH), F32) for _ in range(4)),
            pltpu.SemaphoreType.DMA((RING,)),
        ],
        compiler_params=pltpu.CompilerParams(vmem_limit_bytes=110 * 2**20),
        name="gated_mix_gqa_relu_decode",
    )(*args)
    return (out.reshape(A_x.shape), dx.reshape(A_x.shape),
            dk.reshape(A_k_cache.shape), dv.reshape(A_v_cache.shape),
            dwq.reshape(A_wq.shape), dwo.reshape(A_wo.shape),
            dw1.reshape(B_w1.shape), dw2.reshape(B_w2.shape), dgw)
```

```python
import jax
import jax.numpy as jnp
from jax import lax
import jax.experimental.pallas as pl
import jax.experimental.pallas.tpu as pltpu

F32 = jnp.float32
BF16 = jnp.bfloat16

NB, D, HQ, HKV, SK, DH, DFF = 2, 512, 32, 8, 8192, 128, 1792
REP = HQ // HKV
GW = REP * DH
SCALE = DH ** -0.5

STREAM = SK // 2
KV_VIEW = (2 * NB, HKV, STREAM, DH)
W_ROWS = 112
DWQ_VIEW = (4, D // 4, HQ * DH)
DWO_VIEW = (4, HQ * DH // 4, D)
DW1_VIEW = (4, D // 4, DFF)
DW2_VIEW = (4, DFF // 4, D)
TAIL = 448
RING = 3
STAGE_ROWS = STREAM // 2
STAGED = 5

NN = (((1,), (0,)), ((), ()))
NT = (((1,), (1,)), ((), ()))
TN = (((0,), (0,)), ((), ()))
ALL = slice(None)


def _dot(a, b, dims):
    return lax.dot_general(a, b, dims, preferred_element_type=F32)


def _blk(i, n):
    return pl.ds(pl.multiple_of(i * n, n), n)


def _loop(lo, hi, body):
    def step(i, carry):
        body(i)
        return carry
    lax.fori_loop(lo, hi, step, 0)


def _start(copies):
    for c in copies:
        c.start()


def _wait(copies):
    for c in copies:
        c.wait()


def _kernel(x_hbm, k_hbm, v_hbm, wq_hbm, wo_hbm, w1_hbm, w2_hbm, gw_hbm, go_hbm,
            out_hbm, dx_hbm, dk_hbm, dv_hbm, dwq_hbm, dwo_hbm, dw1_hbm, dw2_hbm, dgw_hbm,
            k_ref, v_ref, wq_ref, wo_ref, w1_ref, w2_ref, dwq_ref, dwo_ref, dw1_ref, dw2_ref,
            x_ref, gw_ref, go_ref, out_ref, dx_ref, dgw_ref,
            s_ref, dp_ref, ps_ref, q_ref, do_ref, o_ref, dq_ref, stage_ref, sems):
    copy = pltpu.make_async_copy

    def attn_reads():
        return [copy(src, dst, sems.at[0]) for src, dst in (
            (wq_hbm, wq_ref), (x_hbm, x_ref), (gw_hbm, gw_ref), (go_hbm, go_ref), (wo_hbm, wo_ref))]

    def kv_reads(h):
        heads = [(2 * b + h // 4, pl.ds(2 * (h % 4), 2)) for b in range(NB)]
        return [copy(src.at[i], dst.at[i], sems.at[(h + 1) % RING])
                for src, dst in ((k_hbm, k_ref), (v_hbm, v_ref)) for i in heads]

    def last_kv_reads():
        sem = sems.at[HKV % RING]
        return ([copy(k_hbm.at[i], k_ref.at[i], sem)
                 for i in ((3, 6, pl.ds(STAGE_ROWS, STAGE_ROWS)), (3, 7))]
                + [copy(v_hbm.at[i], v_ref.at[i], sem)
                   for i in ((1, pl.ds(6, 2)), (3, pl.ds(6, 2)))])

    def piece(p):
        return (1 + 2 * (p // 4), 6 + p // 2 % 2, _blk(p % 2, STAGE_ROWS))

    def stage_in(p):
        return copy(k_hbm.at[piece(p)], stage_ref, sems.at[RING])

    def stage_out(p):
        return copy(stage_ref, k_ref.at[piece(p)], sems.at[RING])

    def ffn_reads():
        sem, rows = sems.at[(HKV + 1) % RING], pl.ds(0, DFF - TAIL)
        return [copy(w1_hbm, w1_ref, sem), copy(w2_hbm.at[rows], w2_ref.at[rows], sem)]

    def tail_read():
        rows = pl.ds(DFF - TAIL, TAIL)
        return copy(w2_hbm.at[rows], w2_ref.at[rows], sems.at[(HKV + 2) % RING])

    def write(src, dst, idx):
        return copy(src.at[idx], dst.at[idx], sems.at[HKV % RING])

    def slab_writes(n, act):
        src, dst = ((k_ref, dk_hbm), (v_ref, dv_hbm))[n % 2]
        slab = 2 * (n // 2 % 2) + n // 4
        full, rest = divmod(STREAM, W_ROWS)
        _loop(0, full, lambda j: act([write(src, dst, (slab, ALL, _blk(j, W_ROWS)))]))
        act([write(src, dst, (slab, ALL, pl.ds(full * W_ROWS, rest)))])

    def weight_writes(act):
        def dwq(j):
            return write(dwq_ref, dwq_hbm, (ALL, _blk(lax.div(j, 4), 8), _blk(lax.rem(j, 4), HQ * DH // 4)))

        def dwo(j):
            return write(dwo_ref, dwo_hbm, (ALL, _blk(j, 16)))

        def dw1(j):
            return write(dw1_ref, dw1_hbm, (ALL, _blk(j, 8)))

        def dw2(j):
            return write(dw2_ref, dw2_hbm, (ALL, _blk(j, 32)))

        _loop(0, DWO_VIEW[1] // 16, lambda j: act([dwq(j), dwo(j)]))
        _loop(0, DW2_VIEW[1] // 32, lambda j: act([dw1(j), dw2(j)]))
        _loop(DW2_VIEW[1] // 32, DW1_VIEW[1] // 8, lambda j: act([dw1(j)]))

    def small_writes():
        return [copy(src, dst, sems.at[HKV % RING]) for src, dst in (
            (out_ref, out_hbm), (dx_ref, dx_hbm), (dgw_ref, dgw_hbm))]

    _start(attn_reads())
    stage_in(0).start()
    for h in range(RING - 1):
        _start(kv_reads(h))
    _wait(attn_reads())
    _start(kv_reads(RING - 1))
    stage_in(0).wait()
    stage_out(0).start()

    x = x_ref[...].astype(F32)
    go = go_ref[...].astype(F32)
    gw = gw_ref[...].astype(F32).reshape(1, D)
    g = jax.nn.sigmoid(jnp.sum(x * gw, axis=-1, keepdims=True))

    row = lax.broadcasted_iota(jnp.int32, (8, D), 0)
    tok0 = row < REP
    first = row % REP == 0

    def spread(t):
        return jnp.where(tok0, jnp.broadcast_to(t[0:1], (8, D)), jnp.broadcast_to(t[1:2], (8, D)))

    def per_token(t):
        return jnp.concatenate([jnp.sum(jnp.where(tok0, t, 0.0), axis=0, keepdims=True),
                                jnp.sum(jnp.where(tok0, 0.0, t), axis=0, keepdims=True)], axis=0)

    x8 = spread(x)
    db8 = spread((1.0 - g) * go)
    x8b = x8.astype(BF16)
    da8b = spread(g * go).astype(BF16)

    own = lax.broadcasted_iota(jnp.int32, (8, GW), 1) // DH == row % REP

    def gather_heads(t):
        t = jnp.where(own, t, 0.0)
        return sum(t[:, i * DH:(i + 1) * DH] for i in range(1, REP)) + t[:, :DH]

    def scatter_heads(t):
        return jnp.where(own, jnp.concatenate([t] * REP, axis=1), 0.0)

    def project(h):
        cols = _blk(h, GW)
        q_ref[h] = gather_heads(_dot(x8b, wq_ref[:, cols], NN))
        do_ref[h] = gather_heads(_dot(da8b, wo_ref[cols, :], NT))
    _loop(0, HKV, project)

    def attend(h):
        last = HKV - 1
        pl.when(h < last)(lambda: _wait(kv_reads(h)))
        pl.when(h + RING < last)(lambda: _start(kv_reads(jnp.minimum(h + RING, last - 1))))
        pl.when(h + RING == last)(lambda: _start(last_kv_reads()))
        pl.when(h + RING == last + 1)(lambda: _start(ffn_reads()))
        pl.when(h + RING == last + 2)(lambda: tail_read().start())

        @pl.when(h % 2 == 0)
        def _():
            stage_out(h // 2).wait()
            stage_in(h // 2 + 1).start()

        @pl.when(jnp.logical_and(h % 2 == 1, h < last))
        def _():
            stage_in(h // 2 + 1).wait()
            stage_out(h // 2 + 1).start()

        @pl.when(h == last)
        def _():
            _wait(last_kv_reads())
            _wait(ffn_reads())
            slab_writes(0, _start)
            stage_in(STAGED - 1).wait()
            stage_out(STAGED - 1).start()
            slab_writes(1, _start)
            stage_out(STAGED - 1).wait()
            slab_writes(2, _start)

        def halves(c):
            return [(2 * b + lax.div(h, 4), 2 * lax.rem(h, 4) + c) for b in range(NB)]

        q, do = q_ref[h], do_ref[h]
        qb, dob = q.astype(BF16), do.astype(BF16)

        def scores(c):
            i0, i1 = halves(c)
            m = lax.broadcasted_iota(jnp.int32, (8, STREAM), 0) < REP
            s_ref[:, _blk(c, STREAM)] = jnp.where(m, _dot(qb, k_ref[i0], NT), _dot(qb, k_ref[i1], NT))
            dp_ref[:, _blk(c, STREAM)] = jnp.where(m, _dot(dob, v_ref[i0], NT), _dot(dob, v_ref[i1], NT))
        _loop(0, 2, scores)

        s = s_ref[...] * SCALE
        e = jnp.exp(s - jnp.max(s, axis=-1, keepdims=True))
        p = e * (1.0 / jnp.sum(e, axis=-1, keepdims=True))
        dp = dp_ref[...]
        ds = p * (dp - jnp.sum(p * dp, axis=-1, keepdims=True)) * SCALE
        ps_ref[...] = jnp.concatenate([p, ds], axis=0).astype(BF16)

        m = lax.broadcasted_iota(jnp.int32, (8, DH), 0) < REP
        zero = jnp.zeros((8, DH), F32)
        to_dv0 = jnp.concatenate([jnp.where(m, do, 0.0), zero], axis=0).astype(BF16)
        to_dv1 = jnp.concatenate([jnp.where(m, 0.0, do), zero], axis=0).astype(BF16)
        to_dk0 = jnp.concatenate([zero, jnp.where(m, q, 0.0)], axis=0).astype(BF16)
        to_dk1 = jnp.concatenate([zero, jnp.where(m, 0.0, q)], axis=0).astype(BF16)

        def grads(c, carry):
            o, dq = carry
            i0, i1 = halves(c)
            ps = ps_ref[:, _blk(c, STREAM)]
            o = o + jnp.where(m, _dot(ps, v_ref[i0], NN)[:8], _dot(ps, v_ref[i1], NN)[:8])
            dq = dq + jnp.where(m, _dot(ps, k_ref[i0], NN)[8:], _dot(ps, k_ref[i1], NN)[8:])
            pst = ps.T
            v_ref[i0] = _dot(pst, to_dv0, NN).astype(BF16)
            v_ref[i1] = _dot(pst, to_dv1, NN).astype(BF16)
            k_ref[i0] = _dot(pst, to_dk0, NN).astype(BF16)
            k_ref[i1] = _dot(pst, to_dk1, NN).astype(BF16)
            return o, dq
        o_ref[h], dq_ref[h] = lax.fori_loop(0, 2, grads, (zero, zero))
    _loop(0, HKV, attend)
    slab_writes(3, _start)

    def unproject(h, carry):
        a8, dx8 = carry
        cols = _blk(h, GW)
        o = scatter_heads(o_ref[h]).astype(BF16)
        dq = scatter_heads(dq_ref[h]).astype(BF16)
        per = DWO_VIEW[1] // GW
        dwo_ref[lax.div(h, per), _blk(lax.rem(h, per), GW), :] = _dot(o, da8b, TN).astype(BF16)
        dwq_ref[:, :, cols] = _dot(x8b, dq, TN).astype(BF16).reshape(*DWQ_VIEW[:2], GW)
        return a8 + _dot(o, wo_ref[cols, :], NN), dx8 + _dot(dq, wq_ref[:, cols], NT)
    zero8 = jnp.zeros((8, D), F32)
    a8, dx8 = lax.fori_loop(0, HKV, unproject, (zero8, zero8))
    slab_writes(4, _start)

    tail_read().wait()
    hid = _dot(x8b, w1_ref[...], NN)
    act = jnp.maximum(hid, 0.0).astype(BF16)
    b8 = _dot(act, w2_ref[...], NN)
    slope = jnp.where(hid > 0.0, 1.0, jnp.where(hid == 0.0, 0.5, 0.0))
    dhid = (_dot(db8.astype(BF16), w2_ref[...], NT) * slope).astype(BF16)
    dx8 = dx8 + jnp.where(first, _dot(dhid, w1_ref[...], NT), 0.0)
    dw1_ref[...] = _dot(jnp.where(first, x8, 0.0).astype(BF16), dhid, TN).astype(BF16).reshape(DW1_VIEW)
    dw2_ref[...] = _dot(act, jnp.where(first, db8, 0.0).astype(BF16), TN).astype(BF16).reshape(DW2_VIEW)

    a = per_token(a8)
    b = per_token(jnp.where(first, b8, 0.0))
    dz = jnp.sum(go * (a - b), axis=-1, keepdims=True) * g * (1.0 - g)
    out_ref[...] = (g * a + (1.0 - g) * b).astype(BF16)
    dx_ref[...] = (per_token(dx8) + dz * gw).astype(BF16)
    dgw_ref[...] = jnp.sum(dz * x, axis=0).astype(BF16)

    _start(small_writes())
    weight_writes(_start)
    for n in range(5, 8):
        slab_writes(n, _start)

    for n in range(8):
        slab_writes(n, _wait)
    weight_writes(_wait)
    _wait(small_writes())


@jax.jit
def pallas_gated_mix__gqa_block_cached__dense_activation_relu__decode_kernel(
    A_x: jax.Array,
    A_k_cache: jax.Array,
    A_v_cache: jax.Array,
    A_wq: jax.Array,
    A_wo: jax.Array,
    B_x: jax.Array,
    B_w1: jax.Array,
    B_w2: jax.Array,
    gate_w: jax.Array,
    grad_out: jax.Array,
):
    del B_x
    args = (A_x.reshape(NB, D), A_k_cache.reshape(KV_VIEW), A_v_cache.reshape(KV_VIEW),
            A_wq, A_wo, B_w1, B_w2, gate_w, grad_out.reshape(NB, D))
    grads = (KV_VIEW, KV_VIEW, DWQ_VIEW, DWO_VIEW, DW1_VIEW, DW2_VIEW)
    out_shapes = ((NB, D), (NB, D), *grads, gate_w.shape)
    hbm = pl.BlockSpec(memory_space=pltpu.HBM)

    out, dx, dk, dv, dwq, dwo, dw1, dw2, dgw = pl.pallas_call(
        _kernel,
        out_shape=[jax.ShapeDtypeStruct(s, BF16) for s in out_shapes],
        in_specs=[hbm] * len(args),
        out_specs=[hbm] * len(out_shapes),
        scratch_shapes=[
            *(pltpu.VMEM(s, BF16) for s in (
                KV_VIEW, KV_VIEW, A_wq.shape, A_wo.shape, B_w1.shape, B_w2.shape, *grads[2:],
                (NB, D), (D,), (NB, D), (NB, D), (NB, D), (D,))),
            pltpu.VMEM((8, SK), F32), pltpu.VMEM((8, SK), F32), pltpu.VMEM((16, SK), BF16),
            *(pltpu.VMEM((HKV, 8, DH), F32) for _ in range(4)),
            pltpu.SMEM((STAGE_ROWS, DH), BF16),
            pltpu.SemaphoreType.DMA((RING + 1,)),
        ],
        compiler_params=pltpu.CompilerParams(vmem_limit_bytes=110 * 2**20),
        name="gated_mix_gqa_relu_decode",
    )(*args)
    return (out.reshape(A_x.shape), dx.reshape(A_x.shape),
            dk.reshape(A_k_cache.shape), dv.reshape(A_v_cache.shape),
            dwq.reshape(A_wq.shape), dwo.reshape(A_wo.shape),
            dw1.reshape(B_w1.shape), dw2.reshape(B_w2.shape), dgw)
```

```python
import jax
import jax.numpy as jnp
from jax import lax
import jax.experimental.pallas as pl
import jax.experimental.pallas.tpu as pltpu

F32 = jnp.float32
BF16 = jnp.bfloat16

NB, D, HQ, HKV, SK, DH, DFF = 2, 512, 32, 8, 8192, 128, 1792
REP = HQ // HKV
GW = REP * DH
SCALE = DH ** -0.5

STREAM = SK // 2
KV_VIEW = (NB, 2, HKV, STREAM, DH)
WQ_VIEW = (4, D // 4, HQ * DH)
WO_VIEW = (4, HQ * DH // 4, D)
W1_VIEW = (4, D // 4, DFF)
W2_VIEW = (4, DFF // 4, D)

R_ROWS = 80
EARLY = 26
W_ROWS = 112
STAGED = (256, 248, 256, 248, 280)
V_SPLIT = 2304
TAIL = 224

NN = (((1,), (0,)), ((), ()))
NT = (((1,), (1,)), ((), ()))
TN = (((0,), (0,)), ((), ()))
ALL = slice(None)


def _dot(a, b, dims):
    return lax.dot_general(a, b, dims, preferred_element_type=F32)


def _blk(i, n):
    return pl.ds(pl.multiple_of(i * n, n), n)


def _loop(lo, hi, body):
    def step(i, carry):
        body(i)
        return carry
    lax.fori_loop(lo, hi, step, 0)


def _start(copies):
    for c in copies:
        c.start()


def _wait(copies):
    for c in copies:
        c.wait()


def _kernel(x_hbm, k_hbm, v_hbm, wq_hbm, wo_hbm, w1_hbm, w2_hbm, gw_hbm, go_hbm,
            out_hbm, dx_hbm, dk_hbm, dv_hbm, dwq_hbm, dwo_hbm, dw1_hbm, dw2_hbm, dgw_hbm,
            k_ref, v_ref, wq_ref, wo_ref, w1_ref, w2_ref, dwq_ref, dwo_ref, dw1_ref, dw2_ref,
            x_ref, gw_ref, go_ref, out_ref, dx_ref, dgw_ref,
            s_ref, dp_ref, ps_ref, q_ref, do_ref, o_ref, dq_ref, stage_ref, sems):
    def copy(src, dst, sem, idx=None):
        if idx is not None:
            src, dst = src.at[idx], dst.at[idx]
        return pltpu.make_async_copy(src, dst, sems.at[sem])

    def pieces(act, src, dst, streams, lo, hi, n, skip=0, count=None):
        full, rest = divmod(hi - lo, n)
        _loop(skip, full if count is None else count, lambda j: act(
            [copy(src, dst, 0, (*streams, pl.ds(pl.multiple_of(lo + j * n, 8), n)))]))
        if rest and count is None:
            act([copy(src, dst, 0, (*streams, pl.ds(hi - rest, rest)))])

    def pair(m):
        return (ALL, m // 2, pl.ds(4 * (m % 2), 4))

    def spread_reads(i, act, **part):
        if i == 0:
            pieces(act, v_hbm, v_ref, pair(0), 0, STREAM, R_ROWS, **part)
        elif i < 4:
            pieces(act, k_hbm, k_ref, pair(i - 1), 0, STREAM, R_ROWS, **part)
        else:
            pieces(act, k_hbm, k_ref, pair(3), sum(STAGED), STREAM - TAIL, R_ROWS, **part)
            if "count" not in part:
                pieces(act, v_hbm, v_ref, pair(3), V_SPLIT, STREAM, R_ROWS)

    def spread_wait(i):
        ref = v_ref if i == 0 else k_ref
        copy(ref, ref, 0, pair(max(i - 1, 0))).wait()

    def plain_reads(i):
        if i == 0:
            return [copy(wq_hbm, wq_ref, 1), copy(x_hbm, x_ref, 1), copy(gw_hbm, gw_ref, 1),
                    copy(go_hbm, go_ref, 1), copy(wo_hbm, wo_ref, 1)]
        if i < 3:
            return [copy(v_hbm, v_ref, 1, pair(i))]
        return [copy(w1_hbm, w1_ref, 1), copy(w2_hbm, w2_ref, 1),
                copy(v_hbm, v_ref, 1, (*pair(3), pl.ds(0, V_SPLIT)))]

    def tail_read():
        return copy(k_hbm, k_ref, 2, (*pair(3), pl.ds(STREAM - TAIL, TAIL)))

    def stage(n):
        piece = (*pair(3), pl.ds(sum(STAGED[:n // 2]), STAGED[n // 2]))
        smem = stage_ref.at[ALL, ALL, pl.ds(0, STAGED[n // 2])]
        return copy(smem, k_ref.at[piece], 3) if n % 2 else copy(k_hbm.at[piece], smem, 3)

    def stage_next(n):
        stage(n).wait()
        stage(n + 1).start()

    def slab_writes(n, act):
        src, dst = ((k_ref, dk_hbm), (v_ref, dv_hbm))[n % 2]
        pieces(act, src, dst, (n // 2 % 2, n // 4, ALL), 0, STREAM, W_ROWS)

    def weight_writes(act):
        n1, n2 = W1_VIEW[1] // 8, W2_VIEW[1] // 32
        _loop(0, WO_VIEW[1] // 16, lambda j: act([
            copy(dwq_ref, dwq_hbm, 0, (ALL, _blk(lax.div(j, 4), 8), _blk(lax.rem(j, 4), HQ * DH // 4))),
            copy(dwo_ref, dwo_hbm, 0, (ALL, _blk(j, 16)))]))
        _loop(0, n2, lambda j: act([copy(dw1_ref, dw1_hbm, 0, (ALL, _blk(j, 8))),
                                    copy(dw2_ref, dw2_hbm, 0, (ALL, _blk(j, 32)))]))
        _loop(n2, n1, lambda j: act([copy(dw1_ref, dw1_hbm, 0, (ALL, _blk(j, 8)))]))

    def small_writes():
        return [copy(out_ref, out_hbm, 0), copy(dx_ref, dx_hbm, 0), copy(dgw_ref, dgw_hbm, 0)]

    def interval_ends(i):
        stage_next(i)
        if i % 2 == 0:
            spread_wait(i // 2)
            spread_reads(i // 2 + 1, _start, count=EARLY)
        else:
            spread_reads(i // 2 + 1, _start, skip=EARLY)
            _wait(plain_reads(i // 2))
            _start(plain_reads(i // 2 + 1) if i < 7 else [tail_read()])

    def reads_end():
        spread_reads(4, _wait)
        slab_writes(0, _start)
        stage_next(8)
        slab_writes(1, _start)
        tail_read().wait()
        stage(9).wait()
        slab_writes(2, _start)

    spread_reads(0, _start, count=2)
    stage(0).start()
    spread_reads(0, _start, skip=2)
    _start(plain_reads(0))
    interval_ends(0)
    interval_ends(1)

    x = x_ref[...].astype(F32)
    go = go_ref[...].astype(F32)
    gw = gw_ref[...].astype(F32).reshape(1, D)
    g = jax.nn.sigmoid(jnp.sum(x * gw, axis=-1, keepdims=True))

    row = lax.broadcasted_iota(jnp.int32, (8, D), 0)
    tok0 = row < REP
    first = row % REP == 0

    def spread(t):
        return jnp.where(tok0, jnp.broadcast_to(t[0:1], (8, D)), jnp.broadcast_to(t[1:2], (8, D)))

    def per_token(t):
        return jnp.concatenate([jnp.sum(jnp.where(tok0, t, 0.0), axis=0, keepdims=True),
                                jnp.sum(jnp.where(tok0, 0.0, t), axis=0, keepdims=True)], axis=0)

    x8 = spread(x)
    db8 = spread((1.0 - g) * go)
    x8b = x8.astype(BF16)
    da8b = spread(g * go).astype(BF16)

    own = lax.broadcasted_iota(jnp.int32, (8, GW), 1) // DH == row % REP

    def gather_heads(t):
        t = jnp.where(own, t, 0.0)
        return sum(t[:, i * DH:(i + 1) * DH] for i in range(1, REP)) + t[:, :DH]

    def scatter_heads(t):
        return jnp.where(own, jnp.concatenate([t] * REP, axis=1), 0.0)

    def wq_at(h):
        return (ALL, ALL, _blk(h, GW))

    def wo_at(h):
        return (lax.div(h, 2), _blk(lax.rem(h, 2), GW))

    def project(h):
        q_ref[h] = gather_heads(_dot(x8b, wq_ref[wq_at(h)].reshape(D, GW), NN))
        do_ref[h] = gather_heads(_dot(da8b, wo_ref[wo_at(h)], NT))
    _loop(0, HKV, project)

    def attend(h):
        for i in range(6):
            pl.when(h == i)(lambda i=i: interval_ends(i + 2))
        pl.when(h == 6)(reads_end)
        pl.when(h == 7)(lambda: slab_writes(3, _start))

        def halves(c):
            return [(b, lax.div(h, 4), 2 * lax.rem(h, 4) + c) for b in range(NB)]

        q, do = q_ref[h], do_ref[h]
        qb, dob = q.astype(BF16), do.astype(BF16)

        def scores(c):
            i0, i1 = halves(c)
            m = lax.broadcasted_iota(jnp.int32, (8, STREAM), 0) < REP
            s_ref[:, _blk(c, STREAM)] = jnp.where(m, _dot(qb, k_ref[i0], NT), _dot(qb, k_ref[i1], NT))
            dp_ref[:, _blk(c, STREAM)] = jnp.where(m, _dot(dob, v_ref[i0], NT), _dot(dob, v_ref[i1], NT))
        _loop(0, 2, scores)

        s = s_ref[...] * SCALE
        e = jnp.exp(s - jnp.max(s, axis=-1, keepdims=True))
        dp = dp_ref[...]
        inv = 1.0 / jnp.sum(e, axis=-1, keepdims=True)
        delta = jnp.sum(e * dp, axis=-1, keepdims=True) * inv
        p = e * inv
        ps_ref[...] = jnp.concatenate([p, p * (dp - delta) * SCALE], axis=0).astype(BF16)

        m = lax.broadcasted_iota(jnp.int32, (8, DH), 0) < REP
        zero = jnp.zeros((8, DH), F32)
        to_dv0 = jnp.concatenate([jnp.where(m, do, 0.0), zero], axis=0).astype(BF16)
        to_dv1 = jnp.concatenate([jnp.where(m, 0.0, do), zero], axis=0).astype(BF16)
        to_dk0 = jnp.concatenate([zero, jnp.where(m, q, 0.0)], axis=0).astype(BF16)
        to_dk1 = jnp.concatenate([zero, jnp.where(m, 0.0, q)], axis=0).astype(BF16)

        def grads(c, carry):
            o, dq = carry
            i0, i1 = halves(c)
            ps = ps_ref[:, _blk(c, STREAM)]
            o = o + jnp.where(m, _dot(ps, v_ref[i0], NN)[:8], _dot(ps, v_ref[i1], NN)[:8])
            dq = dq + jnp.where(m, _dot(ps, k_ref[i0], NN)[8:], _dot(ps, k_ref[i1], NN)[8:])
            pst = ps.T
            v_ref[i0] = _dot(pst, to_dv0, NN).astype(BF16)
            v_ref[i1] = _dot(pst, to_dv1, NN).astype(BF16)
            k_ref[i0] = _dot(pst, to_dk0, NN).astype(BF16)
            k_ref[i1] = _dot(pst, to_dk1, NN).astype(BF16)
            return o, dq
        o_ref[h], dq_ref[h] = lax.fori_loop(0, 2, grads, (zero, zero))
    _loop(0, HKV, attend)
    slab_writes(4, _start)

    def unproject(h, carry):
        a8, dx8 = carry
        o = scatter_heads(o_ref[h]).astype(BF16)
        dq = scatter_heads(dq_ref[h]).astype(BF16)
        dwo_ref[wo_at(h)] = _dot(o, da8b, TN).astype(BF16)
        dwq_ref[wq_at(h)] = _dot(x8b, dq, TN).astype(BF16).reshape(*WQ_VIEW[:2], GW)
        return (a8 + _dot(o, wo_ref[wo_at(h)], NN),
                dx8 + _dot(dq, wq_ref[wq_at(h)].reshape(D, GW), NT))
    zero8 = jnp.zeros((8, D), F32)
    a8, dx8 = lax.fori_loop(0, HKV, unproject, (zero8, zero8))
    slab_writes(5, _start)

    w1 = w1_ref[...].reshape(D, DFF)
    w2 = w2_ref[...].reshape(DFF, D)
    hid = _dot(x8b, w1, NN)
    act = jnp.maximum(hid, 0.0).astype(BF16)
    b8 = _dot(act, w2, NN)
    slope = jnp.where(hid > 0.0, 1.0, jnp.where(hid == 0.0, 0.5, 0.0))
    dhid = (_dot(db8.astype(BF16), w2, NT) * slope).astype(BF16)
    dx8 = dx8 + jnp.where(first, _dot(dhid, w1, NT), 0.0)
    dw1_ref[...] = _dot(jnp.where(first, x8, 0.0).astype(BF16), dhid, TN).astype(BF16).reshape(W1_VIEW)
    dw2_ref[...] = _dot(act, jnp.where(first, db8, 0.0).astype(BF16), TN).astype(BF16).reshape(W2_VIEW)

    a = per_token(a8)
    b = per_token(jnp.where(first, b8, 0.0))
    dz = jnp.sum(go * (a - b), axis=-1, keepdims=True) * g * (1.0 - g)
    out_ref[...] = (g * a + (1.0 - g) * b).astype(BF16)
    dx_ref[...] = (per_token(dx8) + dz * gw).astype(BF16)
    dgw_ref[...] = jnp.sum(dz * x, axis=0).astype(BF16)

    _start(small_writes())
    weight_writes(_start)
    for n in range(6, 8):
        slab_writes(n, _start)

    for n in range(8):
        slab_writes(n, _wait)
    weight_writes(_wait)
    _wait(small_writes())


@jax.jit
def pallas_gated_mix__gqa_block_cached__dense_activation_relu__decode_kernel(
    A_x: jax.Array,
    A_k_cache: jax.Array,
    A_v_cache: jax.Array,
    A_wq: jax.Array,
    A_wo: jax.Array,
    B_x: jax.Array,
    B_w1: jax.Array,
    B_w2: jax.Array,
    gate_w: jax.Array,
    grad_out: jax.Array,
):
    del B_x
    big = (A_k_cache, A_v_cache, A_wq, A_wo, B_w1, B_w2)
    views = (KV_VIEW, KV_VIEW, WQ_VIEW, WO_VIEW, W1_VIEW, W2_VIEW)
    args = (A_x.reshape(NB, D), *(t.reshape(v) for t, v in zip(big, views)),
            gate_w, grad_out.reshape(NB, D))
    out_shapes = ((NB, D), (NB, D), *views, (D,))
    hbm = pl.BlockSpec(memory_space=pltpu.HBM)

    out, dx, *grads, dgw = pl.pallas_call(
        _kernel,
        out_shape=[jax.ShapeDtypeStruct(s, BF16) for s in out_shapes],
        in_specs=[hbm] * len(args),
        out_specs=[hbm] * len(out_shapes),
        scratch_shapes=[
            *(pltpu.VMEM(s, BF16) for s in (
                *views, *views[2:], (NB, D), (D,), (NB, D), (NB, D), (NB, D), (D,))),
            pltpu.VMEM((8, SK), F32), pltpu.VMEM((8, SK), F32), pltpu.VMEM((16, SK), BF16),
            *(pltpu.VMEM((HKV, 8, DH), F32) for _ in range(4)),
            pltpu.SMEM((NB, 4, max(STAGED), DH), BF16),
            pltpu.SemaphoreType.DMA((4,)),
        ],
        compiler_params=pltpu.CompilerParams(vmem_limit_bytes=110 * 2**20),
        name="gated_mix_gqa_relu_decode",
    )(*args)
    return (out.reshape(A_x.shape), dx.reshape(A_x.shape),
            *(g.reshape(t.shape) for g, t in zip(grads, big)), dgw)
```
